```python
import os as _os
_os.environ.setdefault("JAX_PLATFORMS", "cpu")
import jax
import jax.numpy as jnp

def _softmax(x, axis=-1):
    return jax.nn.softmax(x, axis=axis)
def _gelu(x):
    return jax.nn.gelu(x, approximate=True)
def _silu(x):
    return jax.nn.silu(x)
def _sigmoid(x):
    return jax.nn.sigmoid(x)
def _layernorm(x, axis=-1, eps=1e-5):
    m = jnp.mean(x, axis=axis, keepdims=True)
    v = jnp.var(x, axis=axis, keepdims=True)
    return (x - m) / jnp.sqrt(v + eps)
def _scatter_add(tgt, idx, src, axis=0):
    return tgt.at[idx].add(src)
def _segment_sum(src, seg, n):
    return jax.ops.segment_sum(src, seg, n)
class _Rng:
    def __init__(self, key):
        self._k = key
    def _next(self):
        self._k, sub = jax.random.split(self._k)
        return sub
    def normal(self, shape):
        return jax.random.normal(self._next(), shape, dtype=jnp.bfloat16)
    def randint(self, lo, hi, shape):
        return jax.random.randint(self._next(), shape, lo, hi, dtype=jnp.int32)
    def uniform(self, shape, lo=0.0, hi=1.0):
        return jax.random.uniform(self._next(), shape, jnp.bfloat16, lo, hi)
    def permutation(self, n):
        return jax.random.permutation(self._next(), n)


kernel_name = 'gated_mix__sliding_block__dense_activation_silu__prompt'

def setup_inputs():
    _rng = _Rng(jax.random.key(int.from_bytes(__import__("os").urandom(4), "little")))
    _w = (lambda a: (lambda t: t.astype(jnp.bfloat16) if jnp.issubdtype(t.dtype, jnp.floating) else t)(jnp.asarray(a)))
    def _A_setup():
        B, S, D = 1, 2048, 640
        return {
            "x": _w((lambda *s: _rng.normal(s) * 0.05)(B, S, D)),
            "wqkv": _w((lambda *s: _rng.normal(s) * 0.4)(D, 3 * D)),
            "wo": _w((lambda *s: _rng.normal(s) * 0.05)(D, D)),
        }
    _A_in = _A_setup()

    def _B_setup():
        B, S, D, F = 1, 2048, 640, 1536
        return {
            "x": _w((lambda *s: _rng.normal(s) * 0.05)(B, S, D)),
            "w1": _w((lambda *s: _rng.normal(s) * 1.6)(D, F) * (D ** -0.5)),
            "w2": _w((lambda *s: _rng.normal(s) * 1.6)(F, D) * (F ** -0.5)),
        }
    _B_in = _B_setup()

    return {
        "A_x": _A_in["x"],
        "A_wqkv": _A_in["wqkv"],
        "A_wo": _A_in["wo"],
        "B_x": _B_in["x"],
        "B_w1": _B_in["w1"],
        "B_w2": _B_in["w2"],
        "gate_w": _w((lambda *s: _rng.normal(s) * 0.05)(640) * 16.0),
    }

def reference(A_x, A_wqkv, A_wo, B_x, B_w1, B_w2, gate_w):
    def _A_ref(x, wqkv, wo):
        B, S, D = x.shape
        H = 32; Dh = D // H; W = 256
        qkv = (lambda x, *d: x.transpose(*d))((x @ wqkv).reshape(B, S, 3, H, Dh), 2, 0, 3, 1, 4)
        q, k, v = qkv[0], qkv[1], qkv[2]
        scores = jnp.einsum("bhqd,bhkd->bhqk", q, k) * (Dh ** -0.5)
        idx = jnp.arange(S)
        mask = (idx[:, None] - idx[None, :] >= 0) & (idx[:, None] - idx[None, :] < W)
        scores = jnp.where(mask[None, None], scores, -1e9)
        p = _softmax(scores, axis=-1)
        o = jnp.einsum("bhqk,bhkd->bhqd", p, v)
        return (lambda x, *d: x.transpose(*d))(o, 0, 2, 1, 3).reshape(B, S, D) @ wo

    def _B_ref(x, w1, w2):
        h = jnp.einsum("bsd,df->bsf", x, w1)
        h = _silu(h)
        out = jnp.einsum("bsf,fd->bsd", h, w2)
        return out

    x = A_x
    g = _sigmoid((x * gate_w).sum(-1, keepdims=True))
    a = _A_ref(x, A_wqkv, A_wo)
    b = _B_ref(x, B_w1, B_w2)
    return g * a + (1 - g) * b
```

```python
import functools
import jax
import jax.numpy as jnp
from jax import lax
import jax.experimental.pallas as pl
import jax.experimental.pallas.tpu as pltpu

S = 2048
D = 640
H = 32
DH = 20
W = 256
F = 1536
TB = 256
NEG = -1e30
LOG2E = 1.4426950408889634


def make_kernel(HG, LA, var):
    QB = 128 // HG
    NG = H // HG
    GD = DH * HG
    NB = TB // QB
    WIN = W + QB
    NS = LA + 1
    f32 = jnp.float32
    bf16 = jnp.bfloat16

    def slab_off(g):
        lo = GD * g
        hi = lo + GD
        if lo // 128 == (hi - 1) // 128:
            off = lo // 128 * 128
        else:
            off = lo
        hb = lo - off
        spare = 127 if hb + GD <= 127 else 0
        assert not (hb <= spare < hb + GD)
        return off, hb, spare

    def kernel(x_ref, wqkv_ref, wo_ref, w1_ref, w2_ref, gw_ref, out_ref,
               wvT_ref, k_ref, vt_ref, q_ref, vs_ref, s_ref, m_ref, oT_ref):
        i = pl.program_id(0)
        lane = lax.broadcasted_iota(jnp.int32, (1, 128), 1)

        @pl.when(i == 0)
        def _():
            wvT_ref[...] = wqkv_ref[:, 2 * D:].astype(f32).T.astype(bf16)
            vt_ref[:, TB:] = jnp.zeros((D, TB), f32)
            for g in range(NG):
                _, _, spare = slab_off(g)
                k_ref[g, TB:, :] = jnp.broadcast_to(
                    jnp.where(lane == spare, NEG, 0.0), (TB, 128)).astype(bf16)

        vt_ref[:, :TB] = vt_ref[:, TB:]
        for g in range(NG):
            k_ref[g, :TB, :] = k_ref[g, TB:, :]

        x = x_ref[...]
        qk = jnp.dot(x, wqkv_ref[:, :2 * D], preferred_element_type=f32)
        vT = lax.dot_general(wvT_ref[...], x, (((1,), (1,)), ((), ())),
                             preferred_element_type=f32)
        vt_ref[:, TB:] = vT
        for g in range(NG):
            off, hb, spare = slab_off(g)
            qg = qk[:, off:off + 128] * (DH ** -0.5 * LOG2E)
            q_ref[g] = jnp.where(lane == spare, 1.0, qg).astype(bf16)
            kg = qk[:, D + off:D + off + 128]
            k_ref[g, TB:, :] = jnp.where(lane == spare, 0.0, kg).astype(bf16)

        row = lax.broadcasted_iota(jnp.int32, (QB, 128), 0)
        col = lax.broadcasted_iota(jnp.int32, (QB, 128), 1) % QB
        top_ok = row > col
        bot_ok = row <= col

        tiles = [(g, b) for g in range(NG) for b in range(NB)]

        def prep_v(g):
            vfull = vt_ref[GD * g:GD * (g + 1), :]
            nsh = 128 // QB
            for sh in range(nsh):
                vs_ref[g % 2, sh] = vfull[:, QB * sh:QB * sh + 384 + QB].astype(bf16)

        def stage_a(t):
            g, b = tiles[t]
            off, hb, spare = slab_off(g)
            slot = t % NS
            qb = pltpu.bitcast(q_ref[g, QB * b:QB * (b + 1), :], jnp.uint32)
            parts = []
            for j in range(HG):
                hm = ((lane >= hb + DH * j) & (lane < hb + DH * (j + 1))) | (lane == spare)
                mk = jnp.where(hm, jnp.uint32(0xFFFFFFFF), jnp.uint32(0))
                parts.append(qb & mk)
            qr = pltpu.bitcast(jnp.concatenate(parts, axis=0), bf16)
            kw = k_ref[g, QB * b:QB * b + WIN, :]
            s = lax.dot_general(kw, qr, (((1,), (1,)), ((), ())),
                                preferred_element_type=f32)
            s = jnp.concatenate([
                jnp.where(top_ok, s[:QB], NEG),
                s[QB:W],
                jnp.where(bot_ok, s[W:], NEG)], axis=0)
            s_ref[slot] = s
            m_ref[slot] = jnp.max(s.reshape(WIN // 8, 8, 128), axis=0)

        def stage_b(t):
            g, b = tiles[t]
            slot = t % NS
            m = jnp.max(m_ref[slot], axis=0, keepdims=True)
            p = jnp.exp2(s_ref[slot] - m)
            l = jnp.sum(p, axis=0, keepdims=True)
            a0 = (QB * b) // 128 * 128
            sh = (QB * b - a0) // QB
            vw = vs_ref[g % 2, sh, :, a0:a0 + WIN]
            r = jnp.dot(vw, p.astype(bf16), preferred_element_type=f32)
            oT_ref[b, GD * g:GD * (g + 1), :] = r * (1.0 / l)

        for t in range(LA):
            stage_a(t)
        for t in range(len(tiles)):
            if tiles[t][1] == 0:
                prep_v(tiles[t][0])
            if t + LA < len(tiles):
                stage_a(t + LA)
            stage_b(t)

        dl = lax.broadcasted_iota(jnp.int32, (QB, D), 1)
        jd = (dl // DH) % HG
        os_ = []
        for b in range(NB):
            t = oT_ref[b].T
            o = t[0:QB]
            for j in range(1, HG):
                o = jnp.where(jd == j, t[QB * j:QB * (j + 1)], o)
            os_.append(o.astype(bf16))
        o = jnp.concatenate(os_, axis=0)
        a = jnp.dot(o, wo_ref[...], preferred_element_type=f32)

        h = jnp.dot(x, w1_ref[...], preferred_element_type=f32)
        h = (h * jax.nn.sigmoid(h)).astype(bf16)
        bb = jnp.dot(h, w2_ref[...], preferred_element_type=f32)

        gl = jnp.sum(x.astype(f32) * gw_ref[...].astype(f32), axis=-1, keepdims=True)
        gt = jax.nn.sigmoid(gl)
        out_ref[...] = (gt * a + (1.0 - gt) * bb).astype(out_ref.dtype)

    return kernel, NG, NB, QB, GD, NS


def run(A_x, A_wqkv, A_wo, B_x, B_w1, B_w2, gate_w, HG=4, LA=1, var=0):
    kernel, NG, NB, QB, GD, NS = make_kernel(HG, LA, var)
    x2 = A_x.reshape(S, D)
    gw = gate_w.reshape(1, D)
    full = lambda shape: pl.BlockSpec(shape, lambda i: (0,) * len(shape))
    out = pl.pallas_call(
        kernel,
        grid=(S // TB,),
        in_specs=[
            pl.BlockSpec((TB, D), lambda i: (i, 0)),
            full((D, 3 * D)), full((D, D)), full((D, F)), full((F, D)), full((1, D)),
        ],
        out_specs=pl.BlockSpec((TB, D), lambda i: (i, 0)),
        out_shape=jax.ShapeDtypeStruct((S, D), jnp.bfloat16),
        scratch_shapes=[
            pltpu.VMEM((D, D), jnp.bfloat16),
            pltpu.VMEM((NG, 2 * TB, 128), jnp.bfloat16),
            pltpu.VMEM((D, 2 * TB), jnp.float32),
            pltpu.VMEM((NG, TB, 128), jnp.bfloat16),
            pltpu.VMEM((2, 128 // QB, GD, 384 + QB), jnp.bfloat16),
            pltpu.VMEM((NS, W + QB, 128), jnp.float32),
            pltpu.VMEM((NS, 8, 128), jnp.float32),
            pltpu.VMEM((NB, D, 128), jnp.float32),
        ],
        compiler_params=pltpu.CompilerParams(
            dimension_semantics=("arbitrary",),
            vmem_limit_bytes=100 * 1024 * 1024),
    )(x2, A_wqkv, A_wo, B_w1, B_w2, gw)
    return out.reshape(1, S, D)


@jax.jit
def pallas_gated_mix__sliding_block__dense_activation_silu__prompt_kernel(
    A_x, A_wqkv, A_wo, B_x, B_w1, B_w2, gate_w,
):
    return run(A_x, A_wqkv, A_wo, B_x, B_w1, B_w2, gate_w, HG=2, LA=4)
```

```python
import jax
import jax.numpy as jnp
from jax import lax
import jax.experimental.pallas as pl
import jax.experimental.pallas.tpu as pltpu

S = 2048
D = 640
H = 32
DH = 20
W = 256
F = 1536
TB = 256
NEG = -1e30
LOG2E = 1.4426950408889634

HG = 2
QB = 128 // HG
NG = H // HG
GD = DH * HG
GP = 48
NB = TB // QB
WIN = W + QB
VL = 384 + QB


def _slab(g):
    lo, hi = GD * g, GD * (g + 1)
    off = lo // 128 * 128 if lo // 128 == (hi - 1) // 128 else lo
    hb = lo - off
    spare = 127 if hb + GD <= 127 else 0
    return off, hb, spare


def _make_kernel(LA, order, early_v):
    NS = LA + 1
    f32 = jnp.float32
    bf16 = jnp.bfloat16

    def kernel(x_ref, xn_ref, wqkv_hbm, wo_hbm, w1_hbm, w2_hbm, gw_ref, out_ref,
               wqk_ref, wv_ref, wo_ref, w1_ref, w2_ref, sems,
               wvT_ref, k_ref, vt_ref, q_ref, vs_ref, s_ref, m_ref, oT_ref):
        i = pl.program_id(0)
        lane = lax.broadcasted_iota(jnp.int32, (1, 128), 1)

        cps = [pltpu.make_async_copy(src, dst, sems.at[n]) for n, (src, dst) in enumerate([
            (wqkv_hbm.at[:, pl.ds(2 * D, D)], wv_ref), (wqkv_hbm.at[:, pl.ds(0, 2 * D)], wqk_ref),
            (w1_hbm, w1_ref), (w2_hbm, w2_ref), (wo_hbm, wo_ref)])]

        def project(xb_ref):
            xb = xb_ref[...]
            qk = jnp.dot(xb, wqk_ref[...], preferred_element_type=f32)
            vT = lax.dot_general(wvT_ref[...], xb, (((1,), (1,)), ((), ())),
                                 preferred_element_type=f32)
            return qk, vT

        def prepare(qk, vT):
            vt_ref[:, :TB] = vt_ref[:, TB:]
            vt_ref[:, TB:] = vT
            for g in range(NG):
                off, hb, spare = _slab(g)
                qg = qk[:, off:off + 128] * (DH ** -0.5 * LOG2E)
                q_ref[g] = jnp.where(lane == spare, 1.0, qg).astype(bf16)
                kg = qk[:, D + off:D + off + 128]
                k_ref[g, :TB, :] = k_ref[g, TB:, :]
                k_ref[g, TB:, :] = jnp.where(lane == spare, 0.0, kg).astype(bf16)

        row = lax.broadcasted_iota(jnp.int32, (QB, 128), 0)
        col = lax.broadcasted_iota(jnp.int32, (QB, 128), 1) % QB
        top_ok = row > col
        bot_ok = row <= col

        tiles = [(g, b) for g in range(NG) for b in range(NB)]

        def prep_v(g):
            vfull = vt_ref[GD * g:GD * (g + 1), :]
            for sh in range(128 // QB):
                vv = jnp.concatenate([vfull[:, QB * sh:QB * sh + VL],
                                      jnp.ones((GP - GD, VL), f32)], axis=0)
                vs_ref[g % 2, sh] = vv.astype(bf16)

        def scores(t):
            g, b = tiles[t]
            off, hb, spare = _slab(g)
            qb = pltpu.bitcast(q_ref[g, QB * b:QB * (b + 1), :], jnp.uint32)
            parts = []
            for j in range(HG):
                hm = ((lane >= hb + DH * j) & (lane < hb + DH * (j + 1))) | (lane == spare)
                parts.append(qb & jnp.where(hm, jnp.uint32(0xFFFFFFFF), jnp.uint32(0)))
            qr = pltpu.bitcast(jnp.concatenate(parts, axis=0), bf16)
            kw = k_ref[g, QB * b:QB * b + WIN, :]
            s = lax.dot_general(kw, qr, (((1,), (1,)), ((), ())), preferred_element_type=f32)
            s = jnp.concatenate([jnp.where(top_ok, s[:QB], NEG), s[QB:W],
                                 jnp.where(bot_ok, s[W:], NEG)], axis=0)
            s_ref[t % NS] = s
            m_ref[t % NS] = jnp.max(s.reshape(WIN // 8, 8, 128), axis=0)

        def attend(t):
            g, b = tiles[t]
            m = jnp.max(m_ref[t % NS], axis=0, keepdims=True)
            p = jnp.exp2(s_ref[t % NS] - m)
            a0 = (QB * b) // 128 * 128
            vw = vs_ref[g % 2, (QB * b - a0) // QB, :, a0:a0 + WIN]
            r = jnp.dot(vw, p.astype(bf16), preferred_element_type=f32)
            oT_ref[b, GD * g:GD * (g + 1), :] = r[:GD] * (1.0 / r[GD:GD + 1])

        @pl.when(i == 0)
        def _():
            cps[0].start()
            cps[1].start()
            vt_ref[:, TB:] = jnp.zeros((D, TB), f32)
            for g in range(NG):
                _, _, spare = _slab(g)
                k_ref[g, TB:, :] = jnp.broadcast_to(
                    jnp.where(lane == spare, NEG, 0.0), (TB, 128)).astype(bf16)
            cps[0].wait()
            wvT_ref[...] = wv_ref[...].astype(f32).T.astype(bf16)
            if early_v:
                x0 = x_ref[...]
                vT = lax.dot_general(wvT_ref[...], x0, (((1,), (1,)), ((), ())),
                                     preferred_element_type=f32)
            cps[1].wait()
            for c in cps[2:]:
                c.start()
            if early_v:
                prepare(jnp.dot(x0, wqk_ref[...], preferred_element_type=f32), vT)
            else:
                prepare(*project(x_ref))
            for t in range(LA):
                scores(t)

        for t in range(len(tiles)):
            if tiles[t][1] == 0:
                prep_v(tiles[t][0])
            if t + LA < len(tiles):
                scores(t + LA)
            attend(t)

        def finish(has_next):
            x = x_ref[...]
            st = {}
            for op in order:
                if op == '1':
                    h = jnp.dot(x, w1_ref[...], preferred_element_type=f32)
                    st['h'] = (h * jax.nn.sigmoid(h)).astype(bf16)
                elif op == '2':
                    st['ffn'] = jnp.dot(st['h'], w2_ref[...], preferred_element_type=f32)
                elif op == 'w':
                    jd = (lax.broadcasted_iota(jnp.int32, (QB, D), 1) // DH) % HG
                    os_ = []
                    for b in range(NB):
                        t = oT_ref[b].T
                        o = t[0:QB]
                        for j in range(1, HG):
                            o = jnp.where(jd == j, t[QB * j:QB * (j + 1)], o)
                        os_.append(o.astype(bf16))
                    st['a'] = jnp.dot(jnp.concatenate(os_, axis=0), wo_ref[...],
                                      preferred_element_type=f32)
                elif op == 'P' and has_next:
                    st['p'] = project(xn_ref)
                elif op == 'p' and has_next:
                    prepare(*st['p'])
                elif op == 'S' and has_next:
                    for t in range(LA):
                        scores(t)
            gate = jax.nn.sigmoid(jnp.sum(x.astype(f32) * gw_ref[...].reshape(1, D).astype(f32),
                                          axis=-1, keepdims=True))
            out_ref[...] = (gate * st['a'] + (1.0 - gate) * st['ffn']).astype(out_ref.dtype)

        @pl.when(i == 0)
        def _():
            for c in cps[2:]:
                c.wait()

        last = pl.num_programs(0) - 1

        @pl.when(i < last)
        def _():
            finish(True)

        @pl.when(i == last)
        def _():
            finish(False)

    return kernel, NS


def run(A_x, A_wqkv, A_wo, B_x, B_w1, B_w2, gate_w, LA=7, order='P1p2Sw', early_v=True):
    del B_x
    kernel, NS = _make_kernel(LA, order, early_v)
    hbm = pl.BlockSpec(memory_space=pl.ANY)
    bf16, f32 = jnp.bfloat16, jnp.float32
    out = pl.pallas_call(
        kernel,
        grid=(S // TB,),
        in_specs=[pl.BlockSpec((TB, D), lambda i: (i, 0)),
                  pl.BlockSpec((TB, D), lambda i: (jnp.minimum(i + 1, S // TB - 1), 0)), hbm, hbm, hbm, hbm,
                  pl.BlockSpec((D,), lambda i: (0,))],
        out_specs=pl.BlockSpec((TB, D), lambda i: (i, 0)),
        out_shape=jax.ShapeDtypeStruct((S, D), bf16),
        scratch_shapes=[
            pltpu.VMEM((D, 2 * D), bf16), pltpu.VMEM((D, D), bf16),
            pltpu.VMEM((D, D), bf16), pltpu.VMEM((D, F), bf16), pltpu.VMEM((F, D), bf16),
            pltpu.SemaphoreType.DMA((5,)),
            pltpu.VMEM((D, D), bf16),
            pltpu.VMEM((NG, 2 * TB, 128), bf16),
            pltpu.VMEM((D, 2 * TB), f32),
            pltpu.VMEM((NG, TB, 128), bf16),
            pltpu.VMEM((2, 128 // QB, GP, VL), bf16),
            pltpu.VMEM((NS, WIN, 128), f32),
            pltpu.VMEM((NS, 8, 128), f32),
            pltpu.VMEM((NB, D, 128), f32),
        ],
        compiler_params=pltpu.CompilerParams(
            dimension_semantics=("arbitrary",), vmem_limit_bytes=100 * 1024 * 1024),
    )(A_x.reshape(S, D), A_x.reshape(S, D), A_wqkv, A_wo, B_w1, B_w2, gate_w)
    return out.reshape(1, S, D)


@jax.jit
def pallas_gated_mix__sliding_block__dense_activation_silu__prompt_kernel(
    A_x, A_wqkv, A_wo, B_x, B_w1, B_w2, gate_w,
):
    return run(A_x, A_wqkv, A_wo, B_x, B_w1, B_w2, gate_w, )
```

```python
import jax
import jax.numpy as jnp
from jax import lax
import jax.experimental.pallas as pl
import jax.experimental.pallas.tpu as pltpu

S = 2048
D = 640
H = 32
DH = 20
W = 256
F = 1536
TB = 256
NEG = -1e30
LOG2E = 1.4426950408889634

HG = 2
QB = 128 // HG
NG = H // HG
GD = DH * HG
GP = 48
NB = TB // QB
WIN = W + QB
VL = 384 + QB
LA = 10
NS = LA + 1


def _slab(g):
    lo, hi = GD * g, GD * (g + 1)
    off = lo // 128 * 128 if lo // 128 == (hi - 1) // 128 else lo
    return off, lo - off


def _make_kernel():
    f32 = jnp.float32
    bf16 = jnp.bfloat16

    def kernel(x_ref, xn_ref, wqkv_hbm, wo_hbm, w1_hbm, w2_hbm, gw_ref, out_ref,
               wqk_ref, wv_ref, wo_ref, w1_ref, w2_ref, sems,
               wvT_ref, k_ref, vt_ref, q_ref, vs_ref, s_ref, m_ref, oT_ref):
        i = pl.program_id(0)
        lane = lax.broadcasted_iota(jnp.int32, (1, 128), 1)

        cps = [pltpu.make_async_copy(src, dst, sems.at[n]) for n, (src, dst) in enumerate([
            (wqkv_hbm.at[:, pl.ds(2 * D, D)], wv_ref), (wqkv_hbm.at[:, pl.ds(0, 2 * D)], wqk_ref),
            (w1_hbm, w1_ref), (w2_hbm, w2_ref), (wo_hbm, wo_ref)])]

        def project(xb_ref):
            xb = xb_ref[...]
            qk = jnp.dot(xb, wqk_ref[...], preferred_element_type=f32)
            vT = lax.dot_general(wvT_ref[...], xb, (((1,), (1,)), ((), ())),
                                 preferred_element_type=f32)
            return qk, vT

        def prepare(qk, vT, slide=True):
            if slide:
                vt_ref[:, :TB] = vt_ref[:, TB:]
            vt_ref[:, TB:] = vT
            for g in range(NG):
                off, _ = _slab(g)
                q_ref[g] = (qk[:, off:off + 128] * (DH ** -0.5 * LOG2E)).astype(bf16)
                if slide:
                    k_ref[g, :TB, :] = k_ref[g, TB:, :]
                k_ref[g, TB:, :] = qk[:, D + off:D + off + 128].astype(bf16)

        row = lax.broadcasted_iota(jnp.int32, (QB, 128), 0)
        col = lax.broadcasted_iota(jnp.int32, (QB, 128), 1) % QB
        top_ok = row > col
        bot_ok = row <= col

        tiles = [(g, b) for g in range(NG) for b in range(NB)]

        def prep_v(g, first):
            if first:
                vv = jnp.concatenate([vt_ref[GD * g:GD * (g + 1), TB:],
                                      jnp.ones((GP - GD, TB), f32)], axis=0)
                vs_ref[g % 2, 0, :, :TB] = vv.astype(bf16)
                return
            vfull = vt_ref[GD * g:GD * (g + 1), :]
            for sh in range(128 // QB):
                vv = jnp.concatenate([vfull[:, QB * sh:QB * sh + VL],
                                      jnp.ones((GP - GD, VL), f32)], axis=0)
                vs_ref[g % 2, sh] = vv.astype(bf16)

        def scores(t, first):
            g, b = tiles[t]
            off, hb = _slab(g)
            qb = pltpu.bitcast(q_ref[g, QB * b:QB * (b + 1), :], jnp.uint32)
            parts = []
            for j in range(HG):
                hm = (lane >= hb + DH * j) & (lane < hb + DH * (j + 1))
                parts.append(qb & jnp.where(hm, jnp.uint32(0xFFFFFFFF), jnp.uint32(0)))
            qr = pltpu.bitcast(jnp.concatenate(parts, axis=0), bf16)
            if first:
                n = QB * (b + 1)
                kw = k_ref[g, TB:TB + n, :]
            else:
                n = WIN
                kw = k_ref[g, QB * b:QB * b + WIN, :]
            s = lax.dot_general(kw, qr, (((1,), (1,)), ((), ())), preferred_element_type=f32)
            pieces = [s[:n - QB], jnp.where(bot_ok, s[n - QB:], NEG)]
            if not first:
                pieces = [jnp.where(top_ok, s[:QB], NEG), s[QB:n - QB], pieces[1]]
            s = jnp.concatenate([p for p in pieces if p.shape[0]], axis=0)
            s_ref[t % NS, :n, :] = s
            m_ref[t % NS] = jnp.max(s.reshape(n // 8, 8, 128), axis=0)

        def attend(t, first):
            g, b = tiles[t]
            n = QB * (b + 1) if first else WIN
            m = jnp.max(m_ref[t % NS], axis=0, keepdims=True)
            p = jnp.exp2(s_ref[t % NS, :n, :] - m)
            if first:
                vw = vs_ref[g % 2, 0, :, :n]
            else:
                a0 = (QB * b) // 128 * 128
                vw = vs_ref[g % 2, (QB * b - a0) // QB, :, a0:a0 + WIN]
            r = jnp.dot(vw, p.astype(bf16), preferred_element_type=f32)
            oT_ref[b, GD * g:GD * (g + 1), :] = r[:GD] * (1.0 / r[GD:GD + 1])

        @pl.when(i == 0)
        def _():
            cps[0].start()
            cps[1].start()
            cps[0].wait()
            wvT_ref[...] = wv_ref[...].astype(f32).T.astype(bf16)
            x0 = x_ref[...]
            vT = lax.dot_general(wvT_ref[...], x0, (((1,), (1,)), ((), ())),
                                 preferred_element_type=f32)
            cps[1].wait()
            for c in cps[2:]:
                c.start()
            prepare(jnp.dot(x0, wqk_ref[...], preferred_element_type=f32), vT, slide=False)
            for t in range(LA):
                scores(t, True)

        def attention(first):
            for t in range(len(tiles)):
                if tiles[t][1] == 0:
                    prep_v(tiles[t][0], first)
                if t + LA < len(tiles):
                    scores(t + LA, first)
                attend(t, first)

        @pl.when(i == 0)
        def _():
            attention(True)
            for c in cps[2:]:
                c.wait()

        @pl.when(i > 0)
        def _():
            attention(False)

        def finish(has_next):
            x = x_ref[...]
            if has_next:
                qk_next, vT_next = project(xn_ref)
            h = jnp.dot(x, w1_ref[...], preferred_element_type=f32)
            h = (h * jax.nn.sigmoid(h)).astype(bf16)
            if has_next:
                prepare(qk_next, vT_next)
            ffn = jnp.dot(h, w2_ref[...], preferred_element_type=f32)
            if has_next:
                for t in range(LA):
                    scores(t, False)
            jd = (lax.broadcasted_iota(jnp.int32, (QB, D), 1) // DH) % HG
            os_ = []
            for b in range(NB):
                t = oT_ref[b].T
                o = t[0:QB]
                for j in range(1, HG):
                    o = jnp.where(jd == j, t[QB * j:QB * (j + 1)], o)
                os_.append(o.astype(bf16))
            a = jnp.dot(jnp.concatenate(os_, axis=0), wo_ref[...], preferred_element_type=f32)
            gate = jax.nn.sigmoid(jnp.sum(x.astype(f32) * gw_ref[...].reshape(1, D).astype(f32),
                                          axis=-1, keepdims=True))
            out_ref[...] = (gate * a + (1.0 - gate) * ffn).astype(out_ref.dtype)

        last = pl.num_programs(0) - 1

        @pl.when(i < last)
        def _():
            finish(True)

        @pl.when(i == last)
        def _():
            finish(False)

    return kernel


def run(A_x, A_wqkv, A_wo, B_x, B_w1, B_w2, gate_w):
    del B_x
    kernel = _make_kernel()
    hbm = pl.BlockSpec(memory_space=pl.ANY)
    bf16, f32 = jnp.bfloat16, jnp.float32
    out = pl.pallas_call(
        kernel,
        grid=(S // TB,),
        in_specs=[pl.BlockSpec((TB, D), lambda i: (i, 0)),
                  pl.BlockSpec((TB, D), lambda i: (jnp.minimum(i + 1, S // TB - 1), 0)), hbm, hbm, hbm, hbm,
                  pl.BlockSpec((D,), lambda i: (0,))],
        out_specs=pl.BlockSpec((TB, D), lambda i: (i, 0)),
        out_shape=jax.ShapeDtypeStruct((S, D), bf16),
        scratch_shapes=[
            pltpu.VMEM((D, 2 * D), bf16), pltpu.VMEM((D, D), bf16),
            pltpu.VMEM((D, D), bf16), pltpu.VMEM((D, F), bf16), pltpu.VMEM((F, D), bf16),
            pltpu.SemaphoreType.DMA((5,)),
            pltpu.VMEM((D, D), bf16),
            pltpu.VMEM((NG, 2 * TB, 128), bf16),
            pltpu.VMEM((D, 2 * TB), f32),
            pltpu.VMEM((NG, TB, 128), bf16),
            pltpu.VMEM((2, 128 // QB, GP, VL), bf16),
            pltpu.VMEM((NS, WIN, 128), f32),
            pltpu.VMEM((NS, 8, 128), f32),
            pltpu.VMEM((NB, D, 128), f32),
        ],
        compiler_params=pltpu.CompilerParams(
            dimension_semantics=("arbitrary",), vmem_limit_bytes=100 * 1024 * 1024),
    )(A_x.reshape(S, D), A_x.reshape(S, D), A_wqkv, A_wo, B_w1, B_w2, gate_w)
    return out.reshape(1, S, D)


@jax.jit
def pallas_gated_mix__sliding_block__dense_activation_silu__prompt_kernel(
    A_x: jax.Array,
    A_wqkv: jax.Array,
    A_wo: jax.Array,
    B_x: jax.Array,
    B_w1: jax.Array,
    B_w2: jax.Array,
    gate_w: jax.Array,
):
    return run(A_x, A_wqkv, A_wo, B_x, B_w1, B_w2, gate_w)
```
